```python
import os as _os
_os.environ.setdefault("JAX_PLATFORMS", "cpu")
import jax
import jax.numpy as jnp

def _softmax(x, axis=-1):
    return jax.nn.softmax(x, axis=axis)
def _gelu(x):
    return jax.nn.gelu(x, approximate=True)
def _silu(x):
    return jax.nn.silu(x)
def _sigmoid(x):
    return jax.nn.sigmoid(x)
def _layernorm(x, axis=-1, eps=1e-5):
    m = jnp.mean(x, axis=axis, keepdims=True)
    v = jnp.var(x, axis=axis, keepdims=True)
    return (x - m) / jnp.sqrt(v + eps)
def _scatter_add(tgt, idx, src, axis=0):
    return tgt.at[idx].add(src)
def _segment_sum(src, seg, n):
    return jax.ops.segment_sum(src, seg, n)
class _Rng:
    def __init__(self, key):
        self._k = key
    def _next(self):
        self._k, sub = jax.random.split(self._k)
        return sub
    def normal(self, shape):
        return jax.random.normal(self._next(), shape, dtype=jnp.bfloat16)
    def randint(self, lo, hi, shape):
        return jax.random.randint(self._next(), shape, lo, hi, dtype=jnp.int32)
    def uniform(self, shape, lo=0.0, hi=1.0):
        return jax.random.uniform(self._next(), shape, jnp.bfloat16, lo, hi)
    def permutation(self, n):
        return jax.random.permutation(self._next(), n)


kernel_name = 'gated_mix__ssm_conv_h3__ssm_conv_h3__prompt'

def setup_inputs():
    _rng = _Rng(jax.random.key(int.from_bytes(__import__("os").urandom(4), "little")))
    _w = (lambda a: (lambda t: t.astype(jnp.bfloat16) if jnp.issubdtype(t.dtype, jnp.floating) else t)(jnp.asarray(a)))
    def _A_setup():
        B, S, D = 1, 2048, 640
        ks = 4
        return {
            "q": _w((lambda *s: _rng.normal(s) * 0.05)(B, S, D)),
            "k": _w((lambda *s: _rng.normal(s) * 0.05)(B, S, D)),
            "v": _w((lambda *s: _rng.normal(s) * 0.05)(B, S, D)),
            "shift_k": _w((lambda *s: _rng.normal(s) * 0.05)(D, ks) * 0.5),
            "ssm_k": _w((lambda *s: _rng.normal(s) * 0.05)(D, S) * (1.0 / S ** 0.5)),
            "ssm_D": _w((lambda *s: _rng.normal(s) * 0.05)(D)),
        }
    _A_in = _A_setup()

    def _B_setup():
        B, S, D = 1, 2048, 640
        ks = 4
        return {
            "q": _w((lambda *s: _rng.normal(s) * 0.05)(B, S, D)),
            "k": _w((lambda *s: _rng.normal(s) * 0.05)(B, S, D)),
            "v": _w((lambda *s: _rng.normal(s) * 0.05)(B, S, D)),
            "shift_k": _w((lambda *s: _rng.normal(s) * 0.05)(D, ks) * 0.5),
            "ssm_k": _w((lambda *s: _rng.normal(s) * 0.05)(D, S) * (1.0 / S ** 0.5)),
            "ssm_D": _w((lambda *s: _rng.normal(s) * 0.05)(D)),
        }
    _B_in = _B_setup()

    return {
        "A_q": _A_in["q"],
        "A_k": _A_in["k"],
        "A_v": _A_in["v"],
        "A_shift_k": _A_in["shift_k"],
        "A_ssm_k": _A_in["ssm_k"],
        "A_ssm_D": _A_in["ssm_D"],
        "B_q": _B_in["q"],
        "B_k": _B_in["k"],
        "B_v": _B_in["v"],
        "B_shift_k": _B_in["shift_k"],
        "B_ssm_k": _B_in["ssm_k"],
        "B_ssm_D": _B_in["ssm_D"],
        "gate_w": _w((lambda *s: _rng.normal(s) * 0.05)(640) * 16.0),
    }

def reference(A_q, A_k, A_v, A_shift_k, A_ssm_k, A_ssm_D, B_q, B_k, B_v, B_shift_k, B_ssm_k, B_ssm_D, gate_w):
    def _A_ref(q, k, v, shift_k, ssm_k, ssm_D):
        B, S, D = q.shape
        ks = shift_k.shape[-1]
        k_pad = jnp.pad(k, ((0, 0), (ks - 1, 0), (0, 0)))
        k_shift = jnp.zeros_like(k)
        for t in range(ks):
            k_shift = k_shift + k_pad[:, t:t + S, :] * shift_k[:, ks - 1 - t][None, None, :]
        kv = k_shift * v
        L = 2 * S
        kv_pad = jnp.pad(kv, ((0, 0), (0, S), (0, 0)))
        kf_pad = jnp.pad(ssm_k, ((0, 0), (0, S)))
        kv_f = (lambda x, axes=(-2,-1): jnp.fft.rfft2(x.astype(jnp.float32), axes=axes))(kv_pad[:, None, :, :], axes=(1, 2))
        kf_f = (lambda x, axes=(-2,-1): jnp.fft.rfft2(x.astype(jnp.float32), axes=axes))(kf_pad[:, None, :], axes=(1, 2))
        kf_f = (lambda x, *d: x.transpose(*d))(kf_f, 1, 2, 0)
        y_f = kv_f * kf_f[None, :, :, :]
        y = (lambda x, s, axes=(-2,-1): jnp.fft.irfft2(x, s=s, axes=axes).astype(jnp.bfloat16))(y_f, (1, L), axes=(1, 2))[:, 0, :S, :]
        y = y + kv * ssm_D[None, None, :]
        return q * y

    def _B_ref(q, k, v, shift_k, ssm_k, ssm_D):
        B, S, D = q.shape
        ks = shift_k.shape[-1]
        k_pad = jnp.pad(k, ((0, 0), (ks - 1, 0), (0, 0)))
        k_shift = jnp.zeros_like(k)
        for t in range(ks):
            k_shift = k_shift + k_pad[:, t:t + S, :] * shift_k[:, ks - 1 - t][None, None, :]
        kv = k_shift * v
        L = 2 * S
        kv_pad = jnp.pad(kv, ((0, 0), (0, S), (0, 0)))
        kf_pad = jnp.pad(ssm_k, ((0, 0), (0, S)))
        kv_f = (lambda x, axes=(-2,-1): jnp.fft.rfft2(x.astype(jnp.float32), axes=axes))(kv_pad[:, None, :, :], axes=(1, 2))
        kf_f = (lambda x, axes=(-2,-1): jnp.fft.rfft2(x.astype(jnp.float32), axes=axes))(kf_pad[:, None, :], axes=(1, 2))
        kf_f = (lambda x, *d: x.transpose(*d))(kf_f, 1, 2, 0)
        y_f = kv_f * kf_f[None, :, :, :]
        y = (lambda x, s, axes=(-2,-1): jnp.fft.irfft2(x, s=s, axes=axes).astype(jnp.bfloat16))(y_f, (1, L), axes=(1, 2))[:, 0, :S, :]
        y = y + kv * ssm_D[None, None, :]
        return q * y

    x = A_q
    g = _sigmoid((x * gate_w).sum(-1, keepdims=True))
    a = _A_ref(x, A_k, A_v, A_shift_k, A_ssm_k, A_ssm_D)
    b = _B_ref(x, B_k, B_v, B_shift_k, B_ssm_k, B_ssm_D)
    return g * a + (1 - g) * b
```

```python
import functools

import numpy as np
import jax
import jax.numpy as jnp
from jax import lax
import jax.experimental.pallas as pl
import jax.experimental.pallas.tpu as pltpu

BLK = 128
LANES = 128


def _dft_mats():
    n = np.arange(BLK)
    k = np.arange(BLK)
    th = 2.0 * np.pi * np.outer(k + 0.5, n) / (2 * BLK)
    f = np.concatenate([np.cos(th), -np.sin(th)], axis=0)
    g = np.concatenate([np.cos(th).T, -np.sin(th).T], axis=1) / BLK
    return f.astype(np.float32), g.astype(np.float32)


def _kernel(q_ref, gw_ref,
            ka_ref, va_ref, ska_ref, ha_ref, da_ref,
            kb_ref, vb_ref, skb_ref, hb_ref, db_ref,
            f_ref, g_ref,
            o_ref,
            gate_scr, kpad_scr, kv_scr, kvb_scr, x_scr, h_scr, z_scr, acc_scr,
            *, S, NB):
    c = pl.program_id(0)
    CH = 256

    @pl.when(c == 0)
    def _():
        def gbody(r, _):
            rows = pl.ds(pl.multiple_of(r * CH, CH), CH)
            logit = jnp.dot(q_ref[rows, :], gw_ref[...],
                            preferred_element_type=jnp.float32)
            gate_scr[rows, :] = jax.nn.sigmoid(logit)
            return 0
        lax.fori_loop(0, S // CH, gbody, 0)

    kidx = lax.broadcasted_iota(jnp.int32, (BLK, LANES), 0)
    sign = jnp.where(kidx % 2 == 0, 1.0, -1.0).astype(jnp.float32)

    def branch(br, k_ref, v_ref, sk_ref, h_ref, d_ref):
        kpad_scr[0:8, :] = jnp.zeros((8, LANES), jnp.float32)

        def cbody(r, _):
            rows = pl.ds(pl.multiple_of(r * CH, CH), CH)
            kpad_scr[pl.ds(pl.multiple_of(r * CH + 8, 8), CH), :] = (
                k_ref[rows, :].astype(jnp.float32))
            return 0
        lax.fori_loop(0, S // CH, cbody, 0)

        sk = sk_ref[...].astype(jnp.float32)

        def kvbody(r, _):
            base = pl.multiple_of(r * CH, CH)
            win = kpad_scr[pl.ds(base, CH + 8), :]
            ks = win[8:8 + CH] * sk[0:1]
            for j in range(1, 4):
                ks = ks + win[8 - j:8 - j + CH] * sk[j:j + 1]
            kv = ks * v_ref[pl.ds(base, CH), :].astype(jnp.float32)
            kvb = kv.astype(jnp.bfloat16)
            kvb_scr[pl.ds(base, CH), :] = kvb
            kv_scr[pl.ds(base, CH), :] = kvb.astype(jnp.float32)
            return 0
        lax.fori_loop(0, S // CH, kvbody, 0)

        def fbody(i, prev):
            rows = pl.ds(pl.multiple_of(i * BLK, BLK), BLK)
            x_scr[i] = jnp.dot(f_ref[...], kvb_scr[rows, :],
                               preferred_element_type=jnp.float32)
            hf = lax.dot_general(f_ref[...], h_ref[:, rows],
                                 (((1,), (1,)), ((), ())),
                                 preferred_element_type=jnp.float32)
            pr, pi = prev
            hr, hi = hf[:BLK], hf[BLK:]
            h_scr[i, :BLK] = hr - sign * pi
            h_scr[i, BLK:] = hi + sign * pr
            return hr, hi
        zero = jnp.zeros((BLK, LANES), jnp.float32)
        lax.fori_loop(0, NB, fbody, (zero, zero))

        T = 16
        GRP = 4

        def conv_tile(t, _):
            r0 = pl.multiple_of(t * T, T)
            re = pl.ds(r0, T)
            im = pl.ds(r0 + BLK, T)
            for g0 in range(0, NB, GRP):
                accr = [None] * GRP
                acci = [None] * GRP
                for m in range(g0 + GRP):
                    hr = h_scr[m, re, :]
                    hi = h_scr[m, im, :]
                    for u in range(GRP):
                        i = g0 + u
                        if i - m < 0:
                            continue
                        xr = x_scr[i - m, re, :]
                        xi = x_scr[i - m, im, :]
                        tr = xr * hr - xi * hi
                        ti = xr * hi + xi * hr
                        accr[u] = tr if accr[u] is None else accr[u] + tr
                        acci[u] = ti if acci[u] is None else acci[u] + ti
                for u in range(GRP):
                    z_scr[g0 + u, re, :] = accr[u].astype(jnp.bfloat16)
                    z_scr[g0 + u, im, :] = acci[u].astype(jnp.bfloat16)
            return 0
        lax.fori_loop(0, BLK // T, conv_tile, 0)

        dvec = d_ref[...].astype(jnp.float32)

        def ibody(i, _):
            rows = pl.ds(pl.multiple_of(i * BLK, BLK), BLK)
            y = jnp.dot(g_ref[...], z_scr[i], preferred_element_type=jnp.float32)
            y = y + kv_scr[rows, :] * dvec
            gt = gate_scr[rows, :]
            if br == 0:
                acc_scr[rows, :] = gt * y
            else:
                qv = q_ref[rows, pl.ds(pl.multiple_of(c * LANES, LANES), LANES)]
                o_ref[rows, :] = (qv.astype(jnp.float32)
                                  * (acc_scr[rows, :] + (1.0 - gt) * y)
                                  ).astype(o_ref.dtype)
            return 0
        lax.fori_loop(0, NB, ibody, 0)

    branch(0, ka_ref, va_ref, ska_ref, ha_ref, da_ref)
    branch(1, kb_ref, vb_ref, skb_ref, hb_ref, db_ref)


@jax.jit
def pallas_gated_mix__ssm_conv_h3__ssm_conv_h3__prompt_kernel(
    A_q: jax.Array,
    A_k: jax.Array,
    A_v: jax.Array,
    A_shift_k: jax.Array,
    A_ssm_k: jax.Array,
    A_ssm_D: jax.Array,
    B_q: jax.Array,
    B_k: jax.Array,
    B_v: jax.Array,
    B_shift_k: jax.Array,
    B_ssm_k: jax.Array,
    B_ssm_D: jax.Array,
    gate_w: jax.Array,
):
    Bsz, S, D = A_q.shape
    assert Bsz == 1 and S % BLK == 0 and D % LANES == 0
    NB = S // BLK

    f_np, g_np = _dft_mats()
    f_mat = jnp.asarray(f_np, dtype=jnp.bfloat16)
    g_mat = jnp.asarray(g_np, dtype=jnp.bfloat16)

    q = A_q.reshape(S, D)
    gw = jnp.broadcast_to(gate_w.reshape(D, 1), (D, LANES))

    def prep(k, v, sk, h, d):
        return (k.reshape(S, D), v.reshape(S, D), sk.T, h, d.reshape(1, D))

    a_args = prep(A_k, A_v, A_shift_k, A_ssm_k, A_ssm_D)
    b_args = prep(B_k, B_v, B_shift_k, B_ssm_k, B_ssm_D)

    col = pl.BlockSpec((S, LANES), lambda c: (0, c))
    br_specs = [
        col, col,
        pl.BlockSpec((4, LANES), lambda c: (0, c)),
        pl.BlockSpec((LANES, S), lambda c: (c, 0)),
        pl.BlockSpec((1, LANES), lambda c: (0, c)),
    ]
    in_specs = (
        [pl.BlockSpec((S, D), lambda c: (0, 0)),
         pl.BlockSpec((D, LANES), lambda c: (0, 0))]
        + br_specs + br_specs
        + [pl.BlockSpec((2 * BLK, BLK), lambda c: (0, 0)),
           pl.BlockSpec((BLK, 2 * BLK), lambda c: (0, 0))]
    )
    scratch = [
        pltpu.VMEM((S, LANES), jnp.float32),
        pltpu.VMEM((S + 8, LANES), jnp.float32),
        pltpu.VMEM((S, LANES), jnp.float32),
        pltpu.VMEM((S, LANES), jnp.bfloat16),
        pltpu.VMEM((NB, 2 * BLK, LANES), jnp.float32),
        pltpu.VMEM((NB, 2 * BLK, LANES), jnp.float32),
        pltpu.VMEM((NB, 2 * BLK, LANES), jnp.bfloat16),
        pltpu.VMEM((S, LANES), jnp.float32),
    ]
    out = pl.pallas_call(
        functools.partial(_kernel, S=S, NB=NB),
        grid=(D // LANES,),
        in_specs=in_specs,
        out_specs=pl.BlockSpec((S, LANES), lambda c: (0, c)),
        out_shape=jax.ShapeDtypeStruct((S, D), A_q.dtype),
        scratch_shapes=scratch,
        compiler_params=pltpu.CompilerParams(
            dimension_semantics=("arbitrary",),
            vmem_limit_bytes=64 * 1024 * 1024,
        ),
    )(q, gw, *a_args, *b_args, f_mat, g_mat)
    return out.reshape(Bsz, S, D)
```

```python
import functools


import numpy as np
import jax
import jax.numpy as jnp
from jax import lax
import jax.experimental.pallas as pl
import jax.experimental.pallas.tpu as pltpu

BLK = 128
LANES = 128
T = 8
GRP = 4
TPI = 1


def _dft_mats():
    n = np.arange(BLK)
    k = np.arange(BLK)
    th = 2.0 * np.pi * np.outer(k + 0.5, n) / (2 * BLK)
    f = np.concatenate([np.cos(th), -np.sin(th)], axis=0)
    g = np.concatenate([np.cos(th).T, -np.sin(th).T], axis=1) / BLK
    return f.astype(np.float32), g.astype(np.float32)


def _pack_np(a):
    u = np.ascontiguousarray(a, dtype=np.float32).view(np.uint32).astype(np.uint64)
    b = ((u + 0x7FFF + ((u >> 16) & 1)) >> 16).astype(np.uint32)
    return (b[0::2] | (b[1::2] << 16)).astype(np.uint32)


def _pk(x):
    return pltpu.bitcast(x, jnp.uint32)


def _upk(x):
    return pltpu.bitcast(x, jnp.bfloat16)


def _kernel(q_hbm, ka_hbm, va_hbm, ha_hbm, kb_hbm, vb_hbm, hb_hbm,
            gw_ref, ska_ref, da_ref, skb_ref, db_ref, f_ref, g_ref,
            o_ref,
            q_buf, k_buf, v_buf, h_buf, sems, qsem,
            gate_scr, kpad_scr, kvw_scr, hst_scr, x_scr, h_scr, z_scr, y_scr,
            *, S, NB, NC):
    c = pl.program_id(0)
    CH = 256
    W = NB * LANES
    slot = c % 2

    k_hbm = (ka_hbm, kb_hbm)
    v_hbm = (va_hbm, vb_hbm)
    h_hbm = (ha_hbm, hb_hbm)
    sk_refs = (ska_ref, skb_ref)
    d_refs = (da_ref, db_ref)

    def copies(tile, sl):
        cols = pl.ds(pl.multiple_of(tile * LANES, LANES), LANES)
        out = {}
        for br in range(2):
            out["h", br] = pltpu.make_async_copy(
                h_hbm[br].at[cols, :], h_buf.at[sl, br], sems.at[sl * 6 + br])
        for br in range(2):
            out["k", br] = pltpu.make_async_copy(
                k_hbm[br].at[:, cols], k_buf.at[sl, br], sems.at[sl * 6 + 2 + 2 * br])
            out["v", br] = pltpu.make_async_copy(
                v_hbm[br].at[:, cols], v_buf.at[sl, br], sems.at[sl * 6 + 3 + 2 * br])
        return out

    qcopy = pltpu.make_async_copy(q_hbm, q_buf, qsem.at[0])

    @pl.when(c == 0)
    def _():
        for cp in copies(0, 0).values():
            cp.start()
        qcopy.start()

    @pl.when(c + 1 < NC)
    def _():
        for cp in copies(c + 1, 1 - slot).values():
            cp.start()

    cur = copies(c, slot)

    def loop(fn, n):
        def body(it, _):
            fn(it)
            return 0
        lax.fori_loop(0, n, body, 0)

    with jax.named_scope("hstack"):
        for br in range(2):
            cur["h", br].wait()

            def hcp(i, br=br):
                base = pl.multiple_of(i * BLK, BLK)
                hst_scr[pl.ds(pl.multiple_of(br * (W // 2) + i * (LANES // 2), LANES // 2),
                              LANES // 2), :] = _pk(h_buf[slot, br, :, pl.ds(base, BLK)])
            loop(hcp, NB)
    with jax.named_scope("fwdh"):
        h_scr[...] = lax.dot_general(
            _upk(f_ref[...]), _upk(hst_scr[...]), (((1,), (1,)), ((), ())),
            preferred_element_type=jnp.float32)

    for br in range(2):
        with jax.named_scope("kcopy"):
            cur["k", br].wait()
            kpad_scr[0:8, :] = jnp.zeros((8, LANES), jnp.float32)

            def cbody(r, br=br):
                rows = pl.ds(pl.multiple_of(r * CH, CH), CH)
                kpad_scr[pl.ds(pl.multiple_of(r * CH + 8, 8), CH), :] = (
                    k_buf[slot, br, rows, :].astype(jnp.float32))
            loop(cbody, S // CH)
        with jax.named_scope("kv"):
            cur["v", br].wait()
            sk = sk_refs[br][...].astype(jnp.float32)

            def kvbody(i, br=br, sk=sk):
                base = pl.multiple_of(i * BLK, BLK)
                ks = kpad_scr[pl.ds(base + 8, BLK), :] * sk[0:1]
                for j in range(1, 4):
                    ks = ks + kpad_scr[pl.ds(base + 8 - j, BLK), :] * sk[j:j + 1]
                kv = ks * v_buf[slot, br, pl.ds(base, BLK), :].astype(jnp.float32)
                kvw_scr[:, pl.ds(pl.multiple_of(br * W + base, LANES), LANES)] = (
                    _pk(kv.astype(jnp.bfloat16)))
            loop(kvbody, NB)

    with jax.named_scope("fwdx"):
        x_scr[...] = jnp.dot(_upk(f_ref[...]), _upk(kvw_scr[...]),
                             preferred_element_type=jnp.float32)

    def conv_tile(br, t):
        def cs(i):
            return slice(br * W + i * LANES, br * W + (i + 1) * LANES)
        dvec = d_refs[br][...].astype(jnp.float32)
        r0 = pl.multiple_of(t * T, T)
        re = pl.ds(r0, T)
        im = pl.ds(r0 + BLK, T)
        kidx = lax.broadcasted_iota(jnp.int32, (T, LANES), 0)
        sign = jnp.where(kidx % 2 == 0, 1.0, -1.0).astype(jnp.float32)
        prev = None
        for g0 in range(0, NB, GRP):
            acc = [None] * GRP
            for m in range(g0 + GRP):
                hr = h_scr[re, cs(m)]
                hi = h_scr[im, cs(m)]
                if m == 0:
                    hr = hr + dvec
                hs = hr + hi
                hd = hi - hr
                for u in range(GRP):
                    i = g0 + u
                    if i - m < 0:
                        continue
                    xr = x_scr[re, cs(i - m)]
                    xi = x_scr[im, cs(i - m)]
                    xs = xr + xi
                    terms = (hr * xs, xr * hd, xi * hs)
                    if acc[u] is None:
                        acc[u] = list(terms)
                    else:
                        acc[u] = [a + tt for a, tt in zip(acc[u], terms)]
            for u in range(GRP):
                yr = acc[u][0] - acc[u][2]
                yi = acc[u][0] + acc[u][1]
                if prev is None:
                    zr, zi = yr, yi
                else:
                    zr = yr - sign * prev[1]
                    zi = yi + sign * prev[0]
                prev = (yr, yi)
                z_scr[re, cs(g0 + u)] = zr
                z_scr[im, cs(g0 + u)] = zi

    with jax.named_scope("conv"):
        for br in range(2):
            def cv(it, br=br):
                for tt in range(TPI):
                    conv_tile(br, it * TPI + tt)
            loop(cv, BLK // T // TPI)

    with jax.named_scope("inv"):
        y_scr[...] = jnp.dot(_upk(g_ref[...]), z_scr[...].astype(jnp.bfloat16),
                             preferred_element_type=jnp.float32)

    @pl.when(c == 0)
    def _():
        qcopy.wait()

        def gbody(r):
            rows = pl.ds(pl.multiple_of(r * CH, CH), CH)
            logit = jnp.dot(q_buf[rows, :], gw_ref[...],
                            preferred_element_type=jnp.float32)
            gate_scr[rows, :] = jax.nn.sigmoid(logit)
        with jax.named_scope("gate"):
            loop(gbody, S // CH)

    def fin(i):
        base = pl.multiple_of(i * BLK, BLK)
        rows = pl.ds(base, BLK)
        gt = gate_scr[rows, :]
        ya = y_scr[:, rows]
        yb = y_scr[:, pl.ds(pl.multiple_of(W + base, LANES), LANES)]
        qv = q_buf[rows, pl.ds(pl.multiple_of(c * LANES, LANES), LANES)]
        o_ref[rows, :] = (qv.astype(jnp.float32)
                          * (yb + gt * (ya - yb))).astype(o_ref.dtype)
    with jax.named_scope("fin"):
        loop(fin, NB)


@jax.jit
def pallas_gated_mix__ssm_conv_h3__ssm_conv_h3__prompt_kernel(
    A_q: jax.Array,
    A_k: jax.Array,
    A_v: jax.Array,
    A_shift_k: jax.Array,
    A_ssm_k: jax.Array,
    A_ssm_D: jax.Array,
    B_q: jax.Array,
    B_k: jax.Array,
    B_v: jax.Array,
    B_shift_k: jax.Array,
    B_ssm_k: jax.Array,
    B_ssm_D: jax.Array,
    gate_w: jax.Array,
):
    Bsz, S, D = A_q.shape
    assert Bsz == 1 and S % BLK == 0 and D % LANES == 0
    NB = S // BLK
    NC = D // LANES
    W = NB * LANES

    f_np, g_np = _dft_mats()
    f_mat = jnp.asarray(_pack_np(f_np))
    g_mat = jnp.asarray(_pack_np(g_np))

    r2 = lambda a: a.reshape(S, D)
    gw = jnp.broadcast_to(gate_w.reshape(D, 1), (D, LANES))

    anyspec = pl.BlockSpec(memory_space=pl.ANY)
    in_specs = (
        [anyspec] * 7
        + [pl.BlockSpec((D, LANES), lambda c: (0, 0)),
           pl.BlockSpec((4, LANES), lambda c: (0, c)),
           pl.BlockSpec((1, LANES), lambda c: (0, c)),
           pl.BlockSpec((4, LANES), lambda c: (0, c)),
           pl.BlockSpec((1, LANES), lambda c: (0, c)),
           pl.BlockSpec((BLK, BLK), lambda c: (0, 0)),
           pl.BlockSpec((BLK // 2, 2 * BLK), lambda c: (0, 0))]
    )
    scratch = [
        pltpu.VMEM((S, D), jnp.bfloat16),
        pltpu.VMEM((2, 2, S, LANES), jnp.bfloat16),
        pltpu.VMEM((2, 2, S, LANES), jnp.bfloat16),
        pltpu.VMEM((2, 2, LANES, S), jnp.bfloat16),
        pltpu.SemaphoreType.DMA((12,)),
        pltpu.SemaphoreType.DMA((1,)),
        pltpu.VMEM((S, LANES), jnp.float32),
        pltpu.VMEM((S + 8, LANES), jnp.float32),
        pltpu.VMEM((BLK // 2, 2 * W), jnp.uint32),
        pltpu.VMEM((W, BLK), jnp.uint32),
        pltpu.VMEM((2 * BLK, 2 * W), jnp.float32),
        pltpu.VMEM((2 * BLK, 2 * W), jnp.float32),
        pltpu.VMEM((2 * BLK, 2 * W), jnp.float32),
        pltpu.VMEM((BLK, 2 * W), jnp.float32),
    ]
    out = pl.pallas_call(
        functools.partial(_kernel, S=S, NB=NB, NC=NC),
        grid=(NC,),
        in_specs=in_specs,
        out_specs=pl.BlockSpec((S, LANES), lambda c: (0, c)),
        out_shape=jax.ShapeDtypeStruct((S, D), A_q.dtype),
        scratch_shapes=scratch,
        compiler_params=pltpu.CompilerParams(
            dimension_semantics=("arbitrary",),
            vmem_limit_bytes=64 * 1024 * 1024,
        ),
    )(r2(A_q), r2(A_k), r2(A_v), A_ssm_k, r2(B_k), r2(B_v), B_ssm_k,
      gw, A_shift_k.T, A_ssm_D.reshape(1, D), B_shift_k.T, B_ssm_D.reshape(1, D),
      f_mat, g_mat)
    return out.reshape(Bsz, S, D)
```

```python
import functools

import numpy as np
import jax
import jax.numpy as jnp
from jax import lax
import jax.experimental.pallas as pl
import jax.experimental.pallas.tpu as pltpu

BLK = 128
LANES = 128
T = 8
GRP = 4


def _dft_mats():
    n = np.arange(BLK)
    k = np.arange(BLK)
    th = 2.0 * np.pi * np.outer(k + 0.5, n) / (2 * BLK)
    f = np.concatenate([np.cos(th), -np.sin(th)], axis=0)
    g = np.concatenate([np.cos(th).T, -np.sin(th).T], axis=1) / BLK
    sg = np.tile((-1.0) ** k, 2)
    f2 = np.concatenate([f, f * sg[:, None]], axis=0)
    g2 = np.concatenate([g, g * sg[None, :]], axis=0)
    return f2.astype(np.float32), g2.astype(np.float32)


def _pack_np(a):
    u = np.ascontiguousarray(a, dtype=np.float32).view(np.uint32).astype(np.uint64)
    b = ((u + 0x7FFF + ((u >> 16) & 1)) >> 16).astype(np.uint32)
    return (b[0::2] | (b[1::2] << 16)).astype(np.uint32)


def _pk(x):
    return pltpu.bitcast(x, jnp.uint32)


def _upk(x):
    return pltpu.bitcast(x, jnp.bfloat16)


def _kernel(q_hbm, ka_hbm, va_hbm, ha_hbm, kb_hbm, vb_hbm, hb_hbm,
            gw_ref, ska_ref, da_ref, skb_ref, db_ref, f_ref, g_ref,
            o_ref,
            q_buf, k_buf, v_buf, h_buf, sems, qsem,
            gate_scr, kpad_scr, kvw_scr, x_scr, h_scr, z_scr, y_scr,
            *, S, NB, NC):
    c = pl.program_id(0)
    CH = 256
    W = NB * LANES
    HB = NB // 2
    slot = c % 2

    k_hbm = (ka_hbm, kb_hbm)
    v_hbm = (va_hbm, vb_hbm)
    h_hbm = (ha_hbm, hb_hbm)
    sk_refs = (ska_ref, skb_ref)
    d_refs = (da_ref, db_ref)

    def col(br, i):
        return ((i % 2) * 2 * HB + br * HB + i // 2) * LANES

    def copies(tile, sl):
        cols = pl.ds(pl.multiple_of(tile * LANES, LANES), LANES)
        out = {}
        for br in range(2):
            out["k", br] = pltpu.make_async_copy(
                k_hbm[br].at[:, cols], k_buf.at[sl, br], sems.at[sl * 6 + 2 + 2 * br])
            out["v", br] = pltpu.make_async_copy(
                v_hbm[br].at[:, cols], v_buf.at[sl, br], sems.at[sl * 6 + 3 + 2 * br])
        for br in range(2):
            out["h", br] = pltpu.make_async_copy(
                h_hbm[br].at[cols, :], h_buf.at[sl, br], sems.at[sl * 6 + br])
        return out

    qcopy = pltpu.make_async_copy(q_hbm, q_buf, qsem.at[0])

    @pl.when(c == 0)
    def _():
        for cp in copies(0, 0).values():
            cp.start()

    cur = copies(c, slot)

    def loop(fn, n):
        def body(it, _):
            fn(it)
            return 0
        lax.fori_loop(0, n, body, 0)

    for br in range(2):
        cur["k", br].wait()
        kpad_scr[0:8, :] = jnp.zeros((8, LANES), jnp.float32)

        def cbody(r, br=br):
            rows = pl.ds(pl.multiple_of(r * CH, CH), CH)
            kpad_scr[pl.ds(pl.multiple_of(r * CH + 8, 8), CH), :] = (
                k_buf[slot, br, rows, :].astype(jnp.float32))
        loop(cbody, S // CH)

        cur["v", br].wait()
        sk = sk_refs[br][...].astype(jnp.float32)

        def kvbody(ip, br=br, sk=sk):
            for par in range(2):
                base = pl.multiple_of((2 * ip + par) * BLK, BLK)
                ks = kpad_scr[pl.ds(base + 8, BLK), :] * sk[0:1]
                for j in range(1, 4):
                    ks = ks + kpad_scr[pl.ds(base + 8 - j, BLK), :] * sk[j:j + 1]
                kv = ks * v_buf[slot, br, pl.ds(base, BLK), :].astype(jnp.float32)
                cstart = pl.multiple_of(col(br, par) + ip * LANES, LANES)
                kvw_scr[:, pl.ds(cstart, LANES)] = _pk(kv.astype(jnp.bfloat16))
        loop(kvbody, HB)

    for br in range(2):
        cur["h", br].wait()

    @pl.when(c == 0)
    def _():
        qcopy.start()

    @pl.when(c + 1 < NC)
    def _():
        for cp in copies(c + 1, 1 - slot).values():
            cp.start()

    fm = [_upk(f_ref[par * BLK:(par + 1) * BLK, :]) for par in range(2)]
    for br in range(2):
        for i in range(NB):
            cc = col(br, i)
            h_scr[:, cc:cc + LANES] = lax.dot_general(
                fm[i % 2], h_buf[slot, br, :, i * BLK:(i + 1) * BLK],
                (((1,), (1,)), ((), ())), preferred_element_type=jnp.float32)
    for par in range(2):
        x_scr[:, par * W:(par + 1) * W] = jnp.dot(
            fm[par], _upk(kvw_scr[:, par * W:(par + 1) * W]),
            preferred_element_type=jnp.float32)

    dv = []
    for br in range(2):
        dfull = d_refs[br][...].astype(jnp.float32).reshape(1, -1)
        dsel = dfull[:, 0:LANES]
        for cc in range(1, NC):
            dsel = jnp.where(c == cc, dfull[:, cc * LANES:(cc + 1) * LANES], dsel)
        dv.append(dsel)

    def conv_tile(br, t):
        def cs(i):
            return slice(col(br, i), col(br, i) + LANES)
        r0 = pl.multiple_of(t * T, T)
        re = pl.ds(r0, T)
        im = pl.ds(r0 + BLK, T)
        prev = None
        for g0 in range(0, NB, GRP):
            acc = [None] * GRP
            for m in range(g0 + GRP):
                hr = h_scr[re, cs(m)]
                hi = h_scr[im, cs(m)]
                if m == 0:
                    hr = hr + dv[br]
                hs = hr + hi
                hd = hi - hr
                for u in range(GRP):
                    i = g0 + u
                    if i - m < 0:
                        continue
                    xr = x_scr[re, cs(i - m)]
                    xi = x_scr[im, cs(i - m)]
                    xs = xr + xi
                    terms = (hr * xs, xr * hd, xi * hs)
                    if acc[u] is None:
                        acc[u] = list(terms)
                    else:
                        acc[u] = [a + tt for a, tt in zip(acc[u], terms)]
            for u in range(GRP):
                yr = acc[u][0] - acc[u][2]
                yi = acc[u][0] + acc[u][1]
                if prev is None:
                    zr, zi = yr, yi
                else:
                    zr = yr - prev[1]
                    zi = yi + prev[0]
                prev = (yr, yi)
                z_scr[re, cs(g0 + u)] = zr
                z_scr[im, cs(g0 + u)] = zi

    for br in range(2):
        loop(lambda t, br=br: conv_tile(br, t), BLK // T)

    for par in range(2):
        y_scr[:, par * W:(par + 1) * W] = jnp.dot(
            _upk(g_ref[par * (BLK // 2):(par + 1) * (BLK // 2), :]),
            z_scr[:, par * W:(par + 1) * W].astype(jnp.bfloat16),
            preferred_element_type=jnp.float32)

    @pl.when(c == 0)
    def _():
        qcopy.wait()

        def gbody(r):
            rows = pl.ds(pl.multiple_of(r * CH, CH), CH)
            gwb = jnp.broadcast_to(gw_ref[...].astype(jnp.float32).reshape(1, -1),
                                   (LANES, gw_ref.shape[0])).astype(jnp.bfloat16)
            logit = lax.dot_general(q_buf[rows, :], gwb, (((1,), (1,)), ((), ())),
                                    preferred_element_type=jnp.float32)
            gate_scr[rows, :] = jax.nn.sigmoid(logit)
        loop(gbody, S // CH)

    def fin(ip):
        for par in range(2):
            base = pl.multiple_of((2 * ip + par) * BLK, BLK)
            rows = pl.ds(base, BLK)
            gt = gate_scr[rows, :]
            ya = y_scr[:, pl.ds(pl.multiple_of(col(0, par) + ip * LANES, LANES), LANES)]
            yb = y_scr[:, pl.ds(pl.multiple_of(col(1, par) + ip * LANES, LANES), LANES)]
            qv = q_buf[rows, pl.ds(pl.multiple_of(c * LANES, LANES), LANES)]
            o_ref[rows, :] = (qv.astype(jnp.float32)
                              * (yb + gt * (ya - yb))).astype(o_ref.dtype)
    loop(fin, HB)


@jax.jit
def pallas_gated_mix__ssm_conv_h3__ssm_conv_h3__prompt_kernel(
    A_q: jax.Array,
    A_k: jax.Array,
    A_v: jax.Array,
    A_shift_k: jax.Array,
    A_ssm_k: jax.Array,
    A_ssm_D: jax.Array,
    B_q: jax.Array,
    B_k: jax.Array,
    B_v: jax.Array,
    B_shift_k: jax.Array,
    B_ssm_k: jax.Array,
    B_ssm_D: jax.Array,
    gate_w: jax.Array,
):
    Bsz, S, D = A_q.shape
    assert Bsz == 1 and S % (GRP * BLK) == 0 and D % LANES == 0
    assert A_shift_k.shape == (D, 4) and B_shift_k.shape == (D, 4)
    NB = S // BLK
    NC = D // LANES
    W = NB * LANES

    f_np, g_np = _dft_mats()
    f_mat = jnp.asarray(_pack_np(f_np))
    g_mat = jnp.asarray(_pack_np(g_np))

    def r2(a):
        return a.reshape(S, D)

    anyspec = pl.BlockSpec(memory_space=pl.ANY)
    in_specs = (
        [anyspec] * 7
        + [pl.BlockSpec((D,), lambda c: (0,)),
           pl.BlockSpec((4, LANES), lambda c: (0, c)),
           pl.BlockSpec((D,), lambda c: (0,)),
           pl.BlockSpec((4, LANES), lambda c: (0, c)),
           pl.BlockSpec((D,), lambda c: (0,)),
           pl.BlockSpec((2 * BLK, BLK), lambda c: (0, 0)),
           pl.BlockSpec((BLK, 2 * BLK), lambda c: (0, 0))]
    )
    scratch = [
        pltpu.VMEM((S, D), A_q.dtype),
        pltpu.VMEM((2, 2, S, LANES), A_k.dtype),
        pltpu.VMEM((2, 2, S, LANES), A_v.dtype),
        pltpu.VMEM((2, 2, LANES, S), A_ssm_k.dtype),
        pltpu.SemaphoreType.DMA((12,)),
        pltpu.SemaphoreType.DMA((1,)),
        pltpu.VMEM((S, LANES), jnp.float32),
        pltpu.VMEM((S + 8, LANES), jnp.float32),
        pltpu.VMEM((BLK // 2, 2 * W), jnp.uint32),
        pltpu.VMEM((2 * BLK, 2 * W), jnp.float32),
        pltpu.VMEM((2 * BLK, 2 * W), jnp.float32),
        pltpu.VMEM((2 * BLK, 2 * W), jnp.float32),
        pltpu.VMEM((BLK, 2 * W), jnp.float32),
    ]
    out = pl.pallas_call(
        functools.partial(_kernel, S=S, NB=NB, NC=NC),
        grid=(NC,),
        in_specs=in_specs,
        out_specs=pl.BlockSpec((S, LANES), lambda c: (0, c)),
        out_shape=jax.ShapeDtypeStruct((S, D), A_q.dtype),
        scratch_shapes=scratch,
        compiler_params=pltpu.CompilerParams(
            dimension_semantics=("arbitrary",),
            vmem_limit_bytes=64 * 1024 * 1024,
        ),
    )(r2(A_q), r2(A_k), r2(A_v), A_ssm_k, r2(B_k), r2(B_v), B_ssm_k,
      gate_w, A_shift_k.T, A_ssm_D, B_shift_k.T, B_ssm_D,
      f_mat, g_mat)
    return out.reshape(Bsz, S, D)
```

```python
import functools

import numpy as np
import jax
import jax.numpy as jnp
from jax import lax
import jax.experimental.pallas as pl
import jax.experimental.pallas.tpu as pltpu

BLK = 128
LANES = 128
T = 8
GRP = 8


def _dft_mats():
    n = np.arange(BLK)
    k = np.arange(BLK)
    th = 2.0 * np.pi * np.outer(k + 0.5, n) / (2 * BLK)
    f = np.concatenate([np.cos(th), -np.sin(th)], axis=0)
    g = np.concatenate([np.cos(th).T, -np.sin(th).T], axis=1) / BLK
    sg = np.tile((-1.0) ** k, 2)
    f2 = np.concatenate([f, f * sg[:, None]], axis=0)
    g2 = np.concatenate([g, g * sg[None, :]], axis=0)
    return f2.astype(np.float32), g2.astype(np.float32)


def _pack_np(a):
    u = np.ascontiguousarray(a, dtype=np.float32).view(np.uint32).astype(np.uint64)
    b = ((u + 0x7FFF + ((u >> 16) & 1)) >> 16).astype(np.uint32)
    return (b[0::2] | (b[1::2] << 16)).astype(np.uint32)


def _pk(x):
    return pltpu.bitcast(x, jnp.uint32)


def _upk(x):
    return pltpu.bitcast(x, jnp.bfloat16)


def _kernel(q_hbm, ka_hbm, va_hbm, ha_hbm, kb_hbm, vb_hbm, hb_hbm,
            gw_ref, ska_ref, da_ref, skb_ref, db_ref, f_ref, g_ref,
            o_ref,
            q_buf, k_buf, v_buf, h_buf, sems, qsem,
            gate_scr, kpad_scr, kvw_scr, x_scr, h_scr, z_scr, y_scr,
            *, S, NB, NC):
    c = pl.program_id(0)
    CH = 256
    W = NB * LANES
    HB = NB // 2
    slot = c % 2

    k_hbm = (ka_hbm, kb_hbm)
    v_hbm = (va_hbm, vb_hbm)
    h_hbm = (ha_hbm, hb_hbm)
    sk_refs = (ska_ref, skb_ref)
    d_refs = (da_ref, db_ref)

    def col(br, i):
        return ((i % 2) * 2 * HB + br * HB + i // 2) * LANES

    def copies(tile, sl):
        cols = pl.ds(pl.multiple_of(tile * LANES, LANES), LANES)
        out = {}
        for br in range(2):
            out["k", br] = pltpu.make_async_copy(
                k_hbm[br].at[:, cols], k_buf.at[sl, br], sems.at[sl * 6 + 2 + 2 * br])
            out["v", br] = pltpu.make_async_copy(
                v_hbm[br].at[:, cols], v_buf.at[sl, br], sems.at[sl * 6 + 3 + 2 * br])
        for br in range(2):
            out["h", br] = pltpu.make_async_copy(
                h_hbm[br].at[cols, :], h_buf.at[sl, br], sems.at[sl * 6 + br])
        return out

    qcopy = pltpu.make_async_copy(q_hbm, q_buf, qsem.at[0])

    @pl.when(c == 0)
    def _():
        for cp in copies(0, 0).values():
            cp.start()

    cur = copies(c, slot)

    def loop(fn, n):
        def body(it, _):
            fn(it)
            return 0
        lax.fori_loop(0, n, body, 0)

    dv = []
    for br in range(2):
        dfull = d_refs[br][...].astype(jnp.float32).reshape(1, -1)
        dsel = dfull[:, 0:LANES]
        for cc in range(1, NC):
            dsel = jnp.where(c == cc, dfull[:, cc * LANES:(cc + 1) * LANES], dsel)
        dv.append(dsel)

    for br in range(2):
        cur["k", br].wait()
        kpad_scr[0:8, :] = jnp.zeros((8, LANES), jnp.float32)

        def cbody(r, br=br):
            rows = pl.ds(pl.multiple_of(r * CH, CH), CH)
            kpad_scr[pl.ds(pl.multiple_of(r * CH + 8, 8), CH), :] = (
                k_buf[slot, br, rows, :].astype(jnp.float32))
        loop(cbody, S // CH)

        cur["v", br].wait()
        sk = sk_refs[br][...].astype(jnp.float32)

        def kvbody(ip, br=br, sk=sk):
            for par in range(2):
                base = pl.multiple_of((2 * ip + par) * BLK, BLK)
                ks = kpad_scr[pl.ds(base + 8, BLK), :] * sk[0:1]
                for j in range(1, 4):
                    ks = ks + kpad_scr[pl.ds(base + 8 - j, BLK), :] * sk[j:j + 1]
                kv = ks * v_buf[slot, br, pl.ds(base, BLK), :].astype(jnp.float32)
                cstart = pl.multiple_of(col(br, par) + ip * LANES, LANES)
                kvw_scr[:, pl.ds(cstart, LANES)] = _pk(kv.astype(jnp.bfloat16))
                y_scr[:, pl.ds(cstart, LANES)] = kv * dv[br]
        loop(kvbody, HB)

    for br in range(2):
        cur["h", br].wait()

    @pl.when(c == 0)
    def _():
        qcopy.start()

    @pl.when(c + 1 < NC)
    def _():
        for cp in copies(c + 1, 1 - slot).values():
            cp.start()

    fm = [_upk(f_ref[par * BLK:(par + 1) * BLK, :]) for par in range(2)]
    for br in range(2):
        for i in range(NB):
            cc = col(br, i)
            h_scr[:, cc:cc + LANES] = lax.dot_general(
                fm[i % 2], h_buf[slot, br, :, i * BLK:(i + 1) * BLK],
                (((1,), (1,)), ((), ())), preferred_element_type=jnp.float32)
    for par in range(2):
        x_scr[:, par * W:(par + 1) * W] = jnp.dot(
            fm[par], _upk(kvw_scr[:, par * W:(par + 1) * W]),
            preferred_element_type=jnp.float32)

    def conv_tile(br, t):
        def cs(i):
            return slice(col(br, i), col(br, i) + LANES)
        r0 = pl.multiple_of(t * T, T)
        re = pl.ds(r0, T)
        im = pl.ds(r0 + BLK, T)
        prev = None
        for g0 in range(0, NB, GRP):
            acc = [None] * GRP
            for m in reversed(range(g0 + GRP)):
                hr = h_scr[re, cs(m)]
                hi = h_scr[im, cs(m)]
                hs = hr + hi
                hd = hi - hr
                for u in range(GRP):
                    i = g0 + u
                    if i - m < 0:
                        continue
                    xr = x_scr[re, cs(i - m)]
                    xi = x_scr[im, cs(i - m)]
                    xs = xr + xi
                    terms = (hr * xs, xr * hd, xi * hs)
                    if acc[u] is None:
                        acc[u] = list(terms)
                    else:
                        acc[u] = [a + tt for a, tt in zip(acc[u], terms)]
            for u in range(GRP):
                yr = acc[u][0] - acc[u][2]
                yi = acc[u][0] + acc[u][1]
                if prev is None:
                    zr, zi = yr, yi
                else:
                    zr = yr - prev[1]
                    zi = yi + prev[0]
                prev = (yr, yi)
                z_scr[re, cs(g0 + u)] = zr
                z_scr[im, cs(g0 + u)] = zi

    for br in range(2):
        loop(lambda t, br=br: conv_tile(br, t), BLK // T)

    for par in range(2):
        y_scr[:, par * W:(par + 1) * W] += jnp.dot(
            _upk(g_ref[par * (BLK // 2):(par + 1) * (BLK // 2), :]),
            z_scr[:, par * W:(par + 1) * W].astype(jnp.bfloat16),
            preferred_element_type=jnp.float32)

    @pl.when(c == 0)
    def _():
        qcopy.wait()

        def gbody(r):
            rows = pl.ds(pl.multiple_of(r * CH, CH), CH)
            gwb = jnp.broadcast_to(gw_ref[...].astype(jnp.float32).reshape(1, -1),
                                   (LANES, gw_ref.shape[0])).astype(jnp.bfloat16)
            logit = lax.dot_general(q_buf[rows, :], gwb, (((1,), (1,)), ((), ())),
                                    preferred_element_type=jnp.float32)
            gate_scr[rows, :] = jax.nn.sigmoid(logit)
        loop(gbody, S // CH)

    def fin(ip):
        for par in range(2):
            base = pl.multiple_of((2 * ip + par) * BLK, BLK)
            rows = pl.ds(base, BLK)
            gt = gate_scr[rows, :]
            ya = y_scr[:, pl.ds(pl.multiple_of(col(0, par) + ip * LANES, LANES), LANES)]
            yb = y_scr[:, pl.ds(pl.multiple_of(col(1, par) + ip * LANES, LANES), LANES)]
            qv = q_buf[rows, pl.ds(pl.multiple_of(c * LANES, LANES), LANES)]
            o_ref[rows, :] = (qv.astype(jnp.float32)
                              * (yb + gt * (ya - yb))).astype(o_ref.dtype)
    loop(fin, HB)


@jax.jit
def pallas_gated_mix__ssm_conv_h3__ssm_conv_h3__prompt_kernel(
    A_q: jax.Array,
    A_k: jax.Array,
    A_v: jax.Array,
    A_shift_k: jax.Array,
    A_ssm_k: jax.Array,
    A_ssm_D: jax.Array,
    B_q: jax.Array,
    B_k: jax.Array,
    B_v: jax.Array,
    B_shift_k: jax.Array,
    B_ssm_k: jax.Array,
    B_ssm_D: jax.Array,
    gate_w: jax.Array,
):
    Bsz, S, D = A_q.shape
    assert Bsz == 1 and S % (GRP * BLK) == 0 and D % LANES == 0
    assert A_shift_k.shape == (D, 4) and B_shift_k.shape == (D, 4)
    NB = S // BLK
    NC = D // LANES
    W = NB * LANES

    f_np, g_np = _dft_mats()
    f_mat = jnp.asarray(_pack_np(f_np))
    g_mat = jnp.asarray(_pack_np(g_np))

    def r2(a):
        return a.reshape(S, D)

    anyspec = pl.BlockSpec(memory_space=pl.ANY)
    in_specs = (
        [anyspec] * 7
        + [pl.BlockSpec((D,), lambda c: (0,)),
           pl.BlockSpec((4, LANES), lambda c: (0, c)),
           pl.BlockSpec((D,), lambda c: (0,)),
           pl.BlockSpec((4, LANES), lambda c: (0, c)),
           pl.BlockSpec((D,), lambda c: (0,)),
           pl.BlockSpec((2 * BLK, BLK), lambda c: (0, 0)),
           pl.BlockSpec((BLK, 2 * BLK), lambda c: (0, 0))]
    )
    scratch = [
        pltpu.VMEM((S, D), A_q.dtype),
        pltpu.VMEM((2, 2, S, LANES), A_k.dtype),
        pltpu.VMEM((2, 2, S, LANES), A_v.dtype),
        pltpu.VMEM((2, 2, LANES, S), A_ssm_k.dtype),
        pltpu.SemaphoreType.DMA((12,)),
        pltpu.SemaphoreType.DMA((1,)),
        pltpu.VMEM((S, LANES), jnp.float32),
        pltpu.VMEM((S + 8, LANES), jnp.float32),
        pltpu.VMEM((BLK // 2, 2 * W), jnp.uint32),
        pltpu.VMEM((2 * BLK, 2 * W), jnp.float32),
        pltpu.VMEM((2 * BLK, 2 * W), jnp.float32),
        pltpu.VMEM((2 * BLK, 2 * W), jnp.float32),
        pltpu.VMEM((BLK, 2 * W), jnp.float32),
    ]
    out = pl.pallas_call(
        functools.partial(_kernel, S=S, NB=NB, NC=NC),
        grid=(NC,),
        in_specs=in_specs,
        out_specs=pl.BlockSpec((S, LANES), lambda c: (0, c)),
        out_shape=jax.ShapeDtypeStruct((S, D), A_q.dtype),
        scratch_shapes=scratch,
        compiler_params=pltpu.CompilerParams(
            dimension_semantics=("arbitrary",),
            vmem_limit_bytes=64 * 1024 * 1024,
        ),
    )(r2(A_q), r2(A_k), r2(A_v), A_ssm_k, r2(B_k), r2(B_v), B_ssm_k,
      gate_w, A_shift_k.T, A_ssm_D, B_shift_k.T, B_ssm_D,
      f_mat, g_mat)
    return out.reshape(Bsz, S, D)
```

```python
import functools

import numpy as np
import jax
import jax.numpy as jnp
from jax import lax
import jax.experimental.pallas as pl
import jax.experimental.pallas.tpu as pltpu

BLK = 128
LANES = 128
T = 8
GRP = 8


def _dft_mats():
    n = np.arange(BLK)
    k = np.arange(BLK)
    th = 2.0 * np.pi * np.outer(k + 0.5, n) / (2 * BLK)
    f = np.concatenate([np.cos(th), -np.sin(th)], axis=0)
    g = np.concatenate([np.cos(th).T, -np.sin(th).T], axis=1) / BLK
    sg = np.tile((-1.0) ** k, 2)
    f2 = np.concatenate([f, f * sg[:, None]], axis=0)
    g2 = np.concatenate([g, g * sg[None, :]], axis=0)
    return f2.astype(np.float32), g2.astype(np.float32)


def _pack_np(a):
    u = np.ascontiguousarray(a, dtype=np.float32).view(np.uint32).astype(np.uint64)
    b = ((u + 0x7FFF + ((u >> 16) & 1)) >> 16).astype(np.uint32)
    return (b[0::2] | (b[1::2] << 16)).astype(np.uint32)


def _upk(x):
    return pltpu.bitcast(x, jnp.bfloat16)


def _kernel(q_hbm, ka_hbm, va_hbm, ha_hbm, kb_hbm, vb_hbm, hb_hbm,
            gw_ref, ska_ref, da_ref, skb_ref, db_ref, f_ref, g_ref,
            o_ref,
            q_buf, k_buf, v_buf, h_buf, sems, qsem,
            gate_scr, kpad_scr, x_scr, h_scr, z_scr, y_scr,
            *, S, NB, NC):
    c = pl.program_id(0)
    CH = 256
    W = NB * LANES
    HB = NB // 2
    slot = c % 2

    k_hbm = (ka_hbm, kb_hbm)
    v_hbm = (va_hbm, vb_hbm)
    h_hbm = (ha_hbm, hb_hbm)
    sk_refs = (ska_ref, skb_ref)
    d_refs = (da_ref, db_ref)

    def col(br, i):
        return ((i % 2) * 2 * HB + br * HB + i // 2) * LANES

    def copies(tile, sl):
        cols = pl.ds(pl.multiple_of(tile * LANES, LANES), LANES)
        out = {}
        for br in range(2):
            out["k", br] = pltpu.make_async_copy(
                k_hbm[br].at[:, cols], k_buf.at[sl, br], sems.at[sl * 6 + 2 + 2 * br])
            out["v", br] = pltpu.make_async_copy(
                v_hbm[br].at[:, cols], v_buf.at[sl, br], sems.at[sl * 6 + 3 + 2 * br])
        for br in range(2):
            out["h", br] = pltpu.make_async_copy(
                h_hbm[br].at[cols, :], h_buf.at[sl, br], sems.at[sl * 6 + br])
        return out

    qcopy = pltpu.make_async_copy(q_hbm, q_buf, qsem.at[0])

    @pl.when(c == 0)
    def _():
        for cp in copies(0, 0).values():
            cp.start()

    cur = copies(c, slot)

    def loop(fn, n):
        def body(it, _):
            fn(it)
            return 0
        lax.fori_loop(0, n, body, 0)

    dv = []
    for br in range(2):
        dfull = d_refs[br][...].astype(jnp.float32).reshape(1, -1)
        dsel = dfull[:, 0:LANES]
        for cc in range(1, NC):
            dsel = jnp.where(c == cc, dfull[:, cc * LANES:(cc + 1) * LANES], dsel)
        dv.append(dsel)

    fm = [_upk(f_ref[par * BLK:(par + 1) * BLK, :]) for par in range(2)]

    for br in range(2):
        cur["k", br].wait()
        kpad_scr[br, 0:8, :] = jnp.zeros((8, LANES), jnp.float32)

        for r in range(S // CH):
            kpad_scr[br, r * CH + 8:(r + 1) * CH + 8, :] = (
                k_buf[slot, br, r * CH:(r + 1) * CH, :].astype(jnp.float32))

        cur["v", br].wait()
        sk = sk_refs[br][...].astype(jnp.float32)

        for i in range(NB):
            base = i * BLK
            ks = kpad_scr[br, base + 8:base + 8 + BLK, :] * sk[0:1]
            for j in range(1, 4):
                ks = ks + kpad_scr[br, base + 8 - j:base + 8 - j + BLK, :] * sk[j:j + 1]
            kv = ks * v_buf[slot, br, base:base + BLK, :].astype(jnp.float32)
            cc = col(br, i)
            y_scr[:, cc:cc + LANES] = kv * dv[br]
            xf = jnp.dot(fm[i % 2], kv.astype(jnp.bfloat16),
                         preferred_element_type=jnp.float32)
            x_scr[0:2 * BLK, cc:cc + LANES] = xf
            x_scr[2 * BLK:3 * BLK, cc:cc + LANES] = xf[:BLK] + xf[BLK:]

    for br in range(2):
        cur["h", br].wait()

    @pl.when(c == 0)
    def _():
        qcopy.start()

    @pl.when(c + 1 < NC)
    def _():
        for cp in copies(c + 1, 1 - slot).values():
            cp.start()

    for br in range(2):
        for i in range(NB):
            cc = col(br, i)
            hf = lax.dot_general(
                fm[i % 2], h_buf[slot, br, :, i * BLK:(i + 1) * BLK],
                (((1,), (1,)), ((), ())), preferred_element_type=jnp.float32)
            h_scr[0:BLK, cc:cc + LANES] = hf[:BLK]
            h_scr[BLK:2 * BLK, cc:cc + LANES] = hf[:BLK] + hf[BLK:]
            h_scr[2 * BLK:3 * BLK, cc:cc + LANES] = hf[BLK:] - hf[:BLK]

    def conv_tile(br, t):
        def cs(i):
            return slice(col(br, i), col(br, i) + LANES)
        r0 = pl.multiple_of(t * T, T)
        re = pl.ds(r0, T)
        im = pl.ds(r0 + BLK, T)
        ex = pl.ds(r0 + 2 * BLK, T)
        prev = None
        for g0 in range(0, NB, GRP):
            acc = [None] * GRP
            for m in reversed(range(g0 + GRP)):
                hr = h_scr[re, cs(m)]
                hs = h_scr[im, cs(m)]
                hd = h_scr[ex, cs(m)]
                for u in range(GRP):
                    i = g0 + u
                    if i - m < 0:
                        continue
                    xr = x_scr[re, cs(i - m)]
                    xi = x_scr[im, cs(i - m)]
                    xs = x_scr[ex, cs(i - m)]
                    terms = (hr * xs, xr * hd, xi * hs)
                    if acc[u] is None:
                        acc[u] = list(terms)
                    else:
                        acc[u] = [a + tt for a, tt in zip(acc[u], terms)]
            for u in range(GRP):
                yr = acc[u][0] - acc[u][2]
                yi = acc[u][0] + acc[u][1]
                if prev is None:
                    zr, zi = yr, yi
                else:
                    zr = yr - prev[1]
                    zi = yi + prev[0]
                prev = (yr, yi)
                z_scr[re, cs(g0 + u)] = zr
                z_scr[im, cs(g0 + u)] = zi

    for br in range(2):
        loop(lambda t, br=br: conv_tile(br, t), BLK // T)

    @pl.when(c == 0)
    def _():
        qcopy.wait()

        def gbody(r):
            rows = pl.ds(pl.multiple_of(r * CH, CH), CH)
            gwb = jnp.broadcast_to(gw_ref[...].astype(jnp.float32).reshape(1, -1),
                                   (LANES, gw_ref.shape[0])).astype(jnp.bfloat16)
            logit = lax.dot_general(q_buf[rows, :], gwb, (((1,), (1,)), ((), ())),
                                    preferred_element_type=jnp.float32)
            gate_scr[rows, :] = jax.nn.sigmoid(logit)
        loop(gbody, S // CH)

    gm = [_upk(g_ref[par * (BLK // 2):(par + 1) * (BLK // 2), :]) for par in range(2)]
    qcols = pl.ds(pl.multiple_of(c * LANES, LANES), LANES)
    for i in range(NB):
        ys = []
        for br in range(2):
            cc = col(br, i)
            ys.append(y_scr[:, cc:cc + LANES] + jnp.dot(
                gm[i % 2], z_scr[:, cc:cc + LANES].astype(jnp.bfloat16),
                preferred_element_type=jnp.float32))
        ya, yb = ys
        rows = slice(i * BLK, (i + 1) * BLK)
        gt = gate_scr[rows, :]
        qv = q_buf[rows, qcols]
        o_ref[rows, :] = (qv.astype(jnp.float32)
                          * (yb + gt * (ya - yb))).astype(o_ref.dtype)


@jax.jit
def pallas_gated_mix__ssm_conv_h3__ssm_conv_h3__prompt_kernel(
    A_q: jax.Array,
    A_k: jax.Array,
    A_v: jax.Array,
    A_shift_k: jax.Array,
    A_ssm_k: jax.Array,
    A_ssm_D: jax.Array,
    B_q: jax.Array,
    B_k: jax.Array,
    B_v: jax.Array,
    B_shift_k: jax.Array,
    B_ssm_k: jax.Array,
    B_ssm_D: jax.Array,
    gate_w: jax.Array,
):
    Bsz, S, D = A_q.shape
    assert Bsz == 1 and S % (GRP * BLK) == 0 and D % LANES == 0
    assert A_shift_k.shape == (D, 4) and B_shift_k.shape == (D, 4)
    NB = S // BLK
    NC = D // LANES
    W = NB * LANES

    f_np, g_np = _dft_mats()
    f_mat = jnp.asarray(_pack_np(f_np))
    g_mat = jnp.asarray(_pack_np(g_np))

    def r2(a):
        return a.reshape(S, D)

    anyspec = pl.BlockSpec(memory_space=pl.ANY)
    in_specs = (
        [anyspec] * 7
        + [pl.BlockSpec((D,), lambda c: (0,)),
           pl.BlockSpec((4, LANES), lambda c: (0, c)),
           pl.BlockSpec((D,), lambda c: (0,)),
           pl.BlockSpec((4, LANES), lambda c: (0, c)),
           pl.BlockSpec((D,), lambda c: (0,)),
           pl.BlockSpec((2 * BLK, BLK), lambda c: (0, 0)),
           pl.BlockSpec((BLK, 2 * BLK), lambda c: (0, 0))]
    )
    scratch = [
        pltpu.VMEM((S, D), A_q.dtype),
        pltpu.VMEM((2, 2, S, LANES), A_k.dtype),
        pltpu.VMEM((2, 2, S, LANES), A_v.dtype),
        pltpu.VMEM((2, 2, LANES, S), A_ssm_k.dtype),
        pltpu.SemaphoreType.DMA((12,)),
        pltpu.SemaphoreType.DMA((1,)),
        pltpu.VMEM((S, LANES), jnp.float32),
        pltpu.VMEM((2, S + 8, LANES), jnp.float32),
        pltpu.VMEM((3 * BLK, 2 * W), jnp.float32),
        pltpu.VMEM((3 * BLK, 2 * W), jnp.float32),
        pltpu.VMEM((2 * BLK, 2 * W), jnp.float32),
        pltpu.VMEM((BLK, 2 * W), jnp.float32),
    ]
    out = pl.pallas_call(
        functools.partial(_kernel, S=S, NB=NB, NC=NC),
        grid=(NC,),
        in_specs=in_specs,
        out_specs=pl.BlockSpec((S, LANES), lambda c: (0, c)),
        out_shape=jax.ShapeDtypeStruct((S, D), A_q.dtype),
        scratch_shapes=scratch,
        compiler_params=pltpu.CompilerParams(
            dimension_semantics=("arbitrary",),
            vmem_limit_bytes=64 * 1024 * 1024,
        ),
    )(r2(A_q), r2(A_k), r2(A_v), A_ssm_k, r2(B_k), r2(B_v), B_ssm_k,
      gate_w, A_shift_k.T, A_ssm_D, B_shift_k.T, B_ssm_D,
      f_mat, g_mat)
    return out.reshape(Bsz, S, D)
```
